```python
import os as _os
_os.environ.setdefault("JAX_PLATFORMS", "cpu")
import jax
import jax.numpy as jnp

def _softmax(x, axis=-1):
    return jax.nn.softmax(x, axis=axis)
def _gelu(x):
    return jax.nn.gelu(x, approximate=True)
def _silu(x):
    return jax.nn.silu(x)
def _sigmoid(x):
    return jax.nn.sigmoid(x)
def _layernorm(x, axis=-1, eps=1e-5):
    m = jnp.mean(x, axis=axis, keepdims=True)
    v = jnp.var(x, axis=axis, keepdims=True)
    return (x - m) / jnp.sqrt(v + eps)
def _scatter_add(tgt, idx, src, axis=0):
    return tgt.at[idx].add(src)
def _segment_sum(src, seg, n):
    return jax.ops.segment_sum(src, seg, n)
class _Rng:
    def __init__(self, key):
        self._k = key
    def _next(self):
        self._k, sub = jax.random.split(self._k)
        return sub
    def normal(self, shape):
        return jax.random.normal(self._next(), shape, dtype=jnp.bfloat16)
    def randint(self, lo, hi, shape):
        return jax.random.randint(self._next(), shape, lo, hi, dtype=jnp.int32)
    def uniform(self, shape, lo=0.0, hi=1.0):
        return jax.random.uniform(self._next(), shape, jnp.bfloat16, lo, hi)
    def permutation(self, n):
        return jax.random.permutation(self._next(), n)


kernel_name = 'standalone__channel_attn_cbam__vision'

def setup_inputs():
    _rng = _Rng(jax.random.key(int.from_bytes(__import__("os").urandom(4), "little")))
    _w = (lambda a: (lambda t: t.astype(jnp.bfloat16) if jnp.issubdtype(t.dtype, jnp.floating) else t)(jnp.asarray(a)))
    H = W = 224
    C = 192
    r = max(C // 4, 1)
    return {
        "x": _w((lambda *s: _rng.normal(s) * 0.2)(1, H, W, C) + (lambda *s: _rng.normal(s) * 0.2)(1, 1, 1, C) * 2.0),
        "w1": _w((lambda *s: _rng.normal(s) * 0.2)(C, r)),
        "w2": _w((lambda *s: _rng.normal(s) * 0.2)(r, C)),
    }

def reference(x, w1, w2):
    B, H, W, C = x.shape
    xf = x.reshape(B, H * W, C)
    gap = jnp.mean(xf, 1)
    gmp = jnp.amax(xf, 1)
    h_a = gap @ w1
    h_a = h_a * (lambda x, dt: x.astype(dt))(h_a > 0, h_a.dtype)
    h_m = gmp @ w1
    h_m = h_m * (lambda x, dt: x.astype(dt))(h_m > 0, h_m.dtype)
    scale = _sigmoid(h_a @ w2 + h_m @ w2)
    return x * scale[:, None, None, :]
```

```python
import jax
import jax.numpy as jnp
from jax import lax
import jax.experimental.pallas as pl
import jax.experimental.pallas.tpu as pltpu

_IN_CHUNKS = (100, 60, 32, 16, 8, 4, 2, 2)
_OUT_CHUNKS = (2, 6, 16, 40, 80, 80)
_CB = 32
_UNROLL = 2


def _kernel(x_hbm, w1t_hbm, w2_hbm, o_hbm,
            xbuf, w1t_v, w2_v, sum_acc, max_acc, scale_v,
            in_sems, out_sems, w_sems):
    H, C, W = xbuf.shape
    cb = _CB
    ncb = C // cb
    in_starts = [sum(_IN_CHUNKS[:i]) for i in range(len(_IN_CHUNKS))]
    out_starts = [sum(_OUT_CHUNKS[:i]) for i in range(len(_OUT_CHUNKS))]

    def in_copy(i):
        sl = pl.ds(in_starts[i], _IN_CHUNKS[i])
        return pltpu.make_async_copy(x_hbm.at[sl], xbuf.at[sl], in_sems.at[i])

    def out_copy(i):
        sl = pl.ds(out_starts[i], _OUT_CHUNKS[i])
        return pltpu.make_async_copy(xbuf.at[sl], o_hbm.at[sl], out_sems.at[i])

    for i in range(len(_IN_CHUNKS)):
        in_copy(i).start()
    w1c = pltpu.make_async_copy(w1t_hbm, w1t_v, w_sems.at[0])
    w2c = pltpu.make_async_copy(w2_hbm, w2_v, w_sems.at[1])
    w1c.start()
    w2c.start()

    for i in range(len(_IN_CHUNKS)):
        in_copy(i).wait()
        h0, n = in_starts[i], _IN_CHUNKS[i]

        def cb_body(j, _, i=i, h0=h0, n=n):
            c0 = pl.multiple_of(j * cb, cb)
            if i == 0:
                v = xbuf[h0, pl.ds(c0, cb), :].astype(jnp.float32)
                init, lo = (v, v), h0 + 1
            else:
                init, lo = (sum_acc[pl.ds(c0, cb), :], max_acc[pl.ds(c0, cb), :]), h0

            def body(h, carry):
                s, m = carry
                v = xbuf[h, pl.ds(c0, cb), :].astype(jnp.float32)
                return s + v, jnp.maximum(m, v)

            s, m = lax.fori_loop(lo, h0 + n, body, init, unroll=_UNROLL)
            sum_acc[pl.ds(c0, cb), :] = s
            max_acc[pl.ds(c0, cb), :] = m
            return 0

        lax.fori_loop(0, ncb, cb_body, 0)

    w1c.wait()
    w2c.wait()
    bf16, f32 = jnp.bfloat16, jnp.float32
    gap = (jnp.sum(sum_acc[...], axis=-1, keepdims=True) * (1.0 / (H * W))).astype(bf16)
    gmp = jnp.max(max_acc[...], axis=-1, keepdims=True).astype(bf16)
    pooled = jnp.concatenate(
        [jnp.broadcast_to(gap, (C, 128)), jnp.broadcast_to(gmp, (C, 128))], axis=-1)
    hid = jnp.dot(w1t_v[...], pooled, preferred_element_type=f32).astype(bf16)
    hid = jnp.maximum(hid.astype(f32), 0.0).astype(bf16)
    y = lax.dot_general(w2_v[...], hid, (((0,), (0,)), ((), ())),
                        preferred_element_type=f32)
    y = y.astype(bf16).astype(f32)
    z = (y[:, :128] + y[:, 128:]).astype(bf16).astype(f32)
    sc = jax.nn.sigmoid(z).astype(bf16).astype(f32)
    scale_v[:, :128] = sc
    scale_v[:, 128:] = sc

    for i in range(len(_OUT_CHUNKS)):
        h0, n = out_starts[i], _OUT_CHUNKS[i]

        def cb_body2(j, _, h0=h0, n=n):
            c0 = pl.multiple_of(j * cb, cb)
            s = scale_v[pl.ds(c0, cb), :W]

            def body(h, _):
                v = xbuf[h, pl.ds(c0, cb), :].astype(jnp.float32)
                xbuf[h, pl.ds(c0, cb), :] = (v * s).astype(xbuf.dtype)
                return 0

            lax.fori_loop(h0, h0 + n, body, 0, unroll=_UNROLL)
            return 0

        lax.fori_loop(0, ncb, cb_body2, 0)
        out_copy(i).start()
    for i in range(len(_OUT_CHUNKS)):
        out_copy(i).wait()


@jax.jit
def pallas_standalone__channel_attn_cbam__vision_kernel(
    x: jax.Array,
    w1: jax.Array,
    w2: jax.Array,
):
    B, H, W, C = x.shape
    r = w1.shape[1]
    assert B == 1 and sum(_IN_CHUNKS) == H and sum(_OUT_CHUNKS) == H
    xt = jnp.transpose(x, (0, 1, 3, 2)).reshape(H, C, W)
    w1t = w1.T
    out = pl.pallas_call(
        _kernel,
        out_shape=jax.ShapeDtypeStruct((H, C, W), x.dtype),
        in_specs=[pl.BlockSpec(memory_space=pl.ANY)] * 3,
        out_specs=pl.BlockSpec(memory_space=pl.ANY),
        scratch_shapes=[
            pltpu.VMEM((H, C, W), x.dtype),
            pltpu.VMEM((r, C), w1.dtype),
            pltpu.VMEM((r, C), w2.dtype),
            pltpu.VMEM((C, W), jnp.float32),
            pltpu.VMEM((C, W), jnp.float32),
            pltpu.VMEM((C, 256), jnp.float32),
            pltpu.SemaphoreType.DMA((len(_IN_CHUNKS),)),
            pltpu.SemaphoreType.DMA((len(_OUT_CHUNKS),)),
            pltpu.SemaphoreType.DMA((2,)),
        ],
        compiler_params=pltpu.CompilerParams(vmem_limit_bytes=64 * 1024 * 1024),
    )(xt, w1t, w2)
    return jnp.transpose(out.reshape(B, H, C, W), (0, 1, 3, 2))
```

```python
import math

import jax
import jax.numpy as jnp
from jax import lax
import jax.experimental.pallas as pl
import jax.experimental.pallas.tpu as pltpu

f32, bf16 = jnp.float32, jnp.bfloat16

_A_CHUNKS = (150, 74)
_B_CHUNKS = (150, 50, 16, 6, 2)
_CB = 32
_ACC_C = 32
_UNROLL1 = 4
_INLINE_MAX = 8
_PARTS = (7,) * 17 + (9,)
_FIRST = (3, 12, 27)
_UNROLL2 = 2


def _starts(chunks):
    return [sum(chunks[:i]) for i in range(len(chunks))]


_PER = sum(_PARTS) * 8


def _kernel(x_hbm, w1t_hbm, w2_hbm, o_hbm,
            xbuf, obuf, w1t_v, w2_v, w1b, w2b, sum_acc, max_acc, scale_v,
            a_sems, b_sems, out_sems, w_sems):
    H, C, W = xbuf.shape
    R = w1t_v.shape[0]
    CA = C - _CB
    inv_n = 1.0 / (H * W)
    NO = o_hbm.shape[0]
    NT = C // math.gcd(_PER, C)
    HG = NT * _PER // C
    a_st, b_st, f_st, p_st = map(_starts, (_A_CHUNKS, _B_CHUNKS, _FIRST, _PARTS))

    def a_copy(i):
        idx = (pl.ds(a_st[i], _A_CHUNKS[i]), pl.ds(0, CA))
        return pltpu.make_async_copy(x_hbm.at[idx], xbuf.at[idx], a_sems.at[i])

    def b_copy(i):
        idx = (pl.ds(b_st[i], _B_CHUNKS[i]), pl.ds(CA, _CB))
        return pltpu.make_async_copy(x_hbm.at[idx], xbuf.at[idx], b_sems.at[i])

    outs = ([(0, f_st[i], _FIRST[i]) for i in range(len(_FIRST))]
            + [(k, 0, NO) for k in range(1, len(_PARTS))])

    def out_copy(i):
        k, o0, n = outs[i]
        idx = (pl.ds(o0, n), pl.ds(p_st[k] * 8, _PARTS[k] * 8))
        return pltpu.make_async_copy(obuf.at[idx], o_hbm.at[idx], out_sems.at[i])

    w1c = pltpu.make_async_copy(w1t_hbm, w1t_v, w_sems.at[0])
    w2c = pltpu.make_async_copy(w2_hbm, w2_v, w_sems.at[1])

    a_copy(0).start()
    w1c.start()
    w2c.start()
    for i in range(1, len(_A_CHUNKS)):
        a_copy(i).start()

    def accum(c0, n_c, lo, hi, carry):
        def body(h, carry):
            s, m = carry
            v = xbuf[h, pl.ds(c0, n_c), :].astype(f32)
            return s + v, jnp.maximum(m, v)

        if hi - lo <= _INLINE_MAX:
            for h in range(lo, hi):
                carry = body(h, carry)
            return carry
        return lax.fori_loop(lo, hi, body, carry, unroll=_UNROLL1)

    def prep_weights():
        w1c.wait()
        w2c.wait()
        row = lax.broadcasted_iota(jnp.int32, (R, 128), 0)
        col = lax.broadcasted_iota(jnp.int32, (R, 128), 1)
        e = jnp.where((col == row) | (col == row + 64), 1.0, 0.0).astype(bf16)
        dn = (((0,), (0,)), ((), ()))
        w1b[...] = lax.dot_general(w1t_v[...], e, dn, preferred_element_type=f32)
        w2b[...] = lax.dot_general(w2_v[...], e, dn, preferred_element_type=f32)

    def layer1_partial(s, m, c0, n_c):
        gap = (jnp.sum(s, axis=-1, keepdims=True) * inv_n).astype(bf16).astype(f32)
        gmp = jnp.max(m, axis=-1, keepdims=True)
        lane = lax.broadcasted_iota(jnp.int32, (n_c, 128), 1)
        prod = jnp.where(lane < 64, gap, gmp) * w1b[pl.ds(c0, n_c), :]
        return jnp.sum(prod.reshape(n_c // 8, 8, 128), axis=0)

    for i in range(len(_A_CHUNKS)):
        a_copy(i).wait()
        if i == 0:
            for j in range(len(_B_CHUNKS)):
                b_copy(j).start()
        h0, n = a_st[i], _A_CHUNKS[i]

        def cb_body(j, _, i=i, h0=h0, n=n):
            c0 = pl.multiple_of(j * _ACC_C, _ACC_C)
            if i == 0:
                v = xbuf[h0, pl.ds(c0, _ACC_C), :].astype(f32)
                init, lo = (v, v), h0 + 1
            else:
                init = (sum_acc[pl.ds(c0, _ACC_C), :], max_acc[pl.ds(c0, _ACC_C), :])
                lo = h0
            s, m = accum(c0, _ACC_C, lo, h0 + n, init)
            sum_acc[pl.ds(c0, _ACC_C), :] = s
            max_acc[pl.ds(c0, _ACC_C), :] = m
            return 0

        lax.fori_loop(0, CA // _ACC_C, cb_body, 0)
    prep_weights()
    part = layer1_partial(sum_acc[...], max_acc[...], 0, CA)

    carry = None
    for i in range(len(_B_CHUNKS)):
        b_copy(i).wait()
        h0, n = b_st[i], _B_CHUNKS[i]
        lo = h0
        if i == 0:
            v = xbuf[h0, pl.ds(CA, _CB), :].astype(f32)
            carry, lo = (v, v), h0 + 1
        carry = accum(CA, _CB, lo, h0 + n, carry)

    part = part + layer1_partial(carry[0], carry[1], CA, _CB)
    hid = jnp.sum(part, axis=0, keepdims=True).astype(bf16).astype(f32)
    hid = jnp.maximum(hid, 0.0)
    z = jnp.sum(w2b[...] * hid, axis=-1, keepdims=True)
    sc = (0.5 * jnp.tanh(0.5 * z) + 0.5).astype(bf16).astype(f32)

    def segments(k, o):
        r, end, segs = p_st[k] * 8, (p_st[k] + _PARTS[k]) * 8, []
        while r < end:
            h, c0 = divmod(o * _PER + r, C)
            n = min(end - r, C - c0)
            segs.append((h, c0, n, r))
            r += n
        return segs

    k, o0, n = outs[0]
    for o in range(o0, o0 + n):
        for (h, c0, nc, r) in segments(k, o):
            v = xbuf[h, pl.ds(c0, nc), :].astype(f32)
            obuf[o, pl.ds(r, nc), :] = (v * sc[c0:c0 + nc]).astype(obuf.dtype)
    out_copy(0).start()
    scale_v[...] = jnp.broadcast_to(sc, (C, 128))
    for i in range(1, len(outs)):
        k, o0, n = outs[i]
        for t in range(NT):
            segs = segments(k, o0 + t)
            ss = []
            for (h, c0, nc, r) in segs:
                s128 = scale_v[pl.ds(c0, nc), :]
                ss.append(jnp.concatenate([s128, s128[:, :W - 128]], axis=1))

            def body(oo, _, segs=segs, ss=ss, o=o0 + t):
                for (h, c0, nc, r), s in zip(segs, ss):
                    v = xbuf[h + HG * oo, pl.ds(c0, nc), :].astype(f32)
                    obuf[o + NT * oo, pl.ds(r, nc), :] = (v * s).astype(obuf.dtype)
                return 0

            lax.fori_loop(0, n // NT, body, 0, unroll=_UNROLL2)
        out_copy(i).start()
    for i in range(len(outs)):
        out_copy(i).wait()


@jax.jit
def pallas_standalone__channel_attn_cbam__vision_kernel(
    x: jax.Array,
    w1: jax.Array,
    w2: jax.Array,
):
    B, H, W, C = x.shape
    r = w1.shape[1]
    NO = H * C // _PER
    NT = C // math.gcd(_PER, C)
    assert B == 1 and r <= 64 and 128 < W <= 256 and NO * _PER == H * C
    assert sum(_A_CHUNKS) == H and sum(_B_CHUNKS) == H and sum(_FIRST) == NO
    assert all(n % NT == 0 for n in _FIRST[1:]) and NO % NT == 0 and (C - _CB) % _ACC_C == 0
    xt = jnp.transpose(x, (0, 1, 3, 2)).reshape(H, C, W)
    out = pl.pallas_call(
        _kernel,
        out_shape=jax.ShapeDtypeStruct((NO, _PER, W), x.dtype),
        in_specs=[pl.BlockSpec(memory_space=pl.ANY)] * 3,
        out_specs=pl.BlockSpec(memory_space=pl.ANY),
        scratch_shapes=[
            pltpu.VMEM((H, C, W), x.dtype),
            pltpu.VMEM((NO, _PER, W), x.dtype),
            pltpu.VMEM((r, C), w1.dtype),
            pltpu.VMEM((r, C), w2.dtype),
            pltpu.VMEM((C, 128), f32),
            pltpu.VMEM((C, 128), f32),
            pltpu.VMEM((C - _CB, W), f32),
            pltpu.VMEM((C - _CB, W), f32),
            pltpu.VMEM((C, 128), f32),
            pltpu.SemaphoreType.DMA((len(_A_CHUNKS),)),
            pltpu.SemaphoreType.DMA((len(_B_CHUNKS),)),
            pltpu.SemaphoreType.DMA((len(_FIRST) + len(_PARTS) - 1,)),
            pltpu.SemaphoreType.DMA((2,)),
        ],
        compiler_params=pltpu.CompilerParams(vmem_limit_bytes=64 * 1024 * 1024),
    )(xt, w1.T, w2)
    return jnp.transpose(out.reshape(B, H, C, W), (0, 1, 3, 2))
```

```python
import jax
import jax.numpy as jnp
from jax import lax
import jax.experimental.pallas as pl
import jax.experimental.pallas.tpu as pltpu

f32, bf16 = jnp.float32, jnp.bfloat16

_F_CHUNKS = (100, 56, 24, 12)
_A_CHUNKS = (16, 10, 6)
_B_CHUNKS = (20, 8, 3, 1)
_CB = 32
_ACC_C = 32
_UNROLL = 4
_INLINE_MAX = 8
_PARTS = (3, 3, 6) + (7,) * 108
_FIRST = (2, 5)
_GROUP = 3
_PER = sum(_PARTS) * 8


def _starts(chunks, base=0):
    return [base + sum(chunks[:i]) for i in range(len(chunks))]


def _kernel(x_hbm, w1t_hbm, w2_hbm, o_hbm,
            xbuf, obuf, w1t_v, w2_v, w1b, w2b, sum_acc, max_acc, scale_v, out_sem):
    H, C, W = xbuf.shape
    R = w1t_v.shape[0]
    CA = C - _CB
    NO = o_hbm.shape[0]
    HG = _PER // C
    HF = sum(_F_CHUNKS)
    p_st = _starts(_PARTS)
    reads = ([(s, n, 0, C) for s, n in zip(_starts(_F_CHUNKS), _F_CHUNKS)]
             + [(s, n, 0, CA) for s, n in zip(_starts(_A_CHUNKS, HF), _A_CHUNKS)]
             + [(s, n, CA, _CB) for s, n in zip(_starts(_B_CHUNKS, HF), _B_CHUNKS)])
    n_fa = len(_F_CHUNKS) + len(_A_CHUNKS)

    def out_copy(k, o0, n):
        idx = (pl.ds(o0, n), pl.ds(p_st[k] * 8, _PARTS[k] * 8))
        return pltpu.make_async_copy(obuf.at[idx], o_hbm.at[idx], out_sem.at[0])

    def accum(c0, n_c, lo, hi, carry):
        def body(h, carry):
            s, m = carry
            v = xbuf[h, pl.ds(c0, n_c), :].astype(f32)
            return s + v, jnp.maximum(m, v)

        if hi - lo <= _INLINE_MAX:
            for h in range(lo, hi):
                carry = body(h, carry)
            return carry
        return lax.fori_loop(lo, hi, body, carry, unroll=_UNROLL)

    def layer1_partial(s, m, c0, n_c):
        gap = (jnp.sum(s, axis=-1, keepdims=True) * (1.0 / (H * W))).astype(bf16).astype(f32)
        gmp = jnp.max(m, axis=-1, keepdims=True)
        lane = lax.broadcasted_iota(jnp.int32, (n_c, 128), 1)
        prod = jnp.where(lane < 64, gap, gmp) * w1b[pl.ds(c0, n_c), :]
        return jnp.sum(prod.reshape(n_c // 8, 8, 128), axis=0)

    def segments(r, end, max_rows):
        segs = []
        while r < end:
            h, c0 = divmod(r, C)
            n = min(end - r, C - c0, max_rows)
            segs.append((h, c0, n, r))
            r += n
        return segs

    def scale_rows(r0, r1):
        for (h, c0, nc, r) in segments(r0, r1, 88):
            s128 = scale_v[pl.ds(c0, nc), :]
            s = jnp.concatenate([s128, s128[:, :W - 128]], axis=1)
            for o in range(NO):
                v = xbuf[h + HG * o, pl.ds(c0, nc), :].astype(f32)
                obuf[o, pl.ds(r, nc), :] = (v * s).astype(obuf.dtype)

    def main(in_sems):
        def in_copy(i):
            h0, n, c0, nc = reads[i]
            idx = (pl.ds(h0, n),) if nc == C else (pl.ds(h0, n), pl.ds(c0, nc))
            return pltpu.make_async_copy(x_hbm.at[idx], xbuf.at[idx], in_sems.at[1 + i])

        w1c = pltpu.make_async_copy(w1t_hbm, w1t_v, in_sems.at[0])
        w2c = pltpu.make_async_copy(w2_hbm, w2_v, in_sems.at[0])
        in_copy(0).start()
        w1c.start()
        w2c.start()
        in_copy(1).start()

        for i in range(n_fa):
            h0, n, _, nc = reads[i]
            in_copy(i).wait()
            if i == 0:
                for j in range(2, len(reads)):
                    in_copy(j).start()

            def cb_body(j, _, i=i, h0=h0, n=n):
                c0 = pl.multiple_of(j * _ACC_C, _ACC_C)
                if i == 0:
                    v = xbuf[h0, pl.ds(c0, _ACC_C), :].astype(f32)
                    init, lo = (v, v), h0 + 1
                else:
                    init = (sum_acc[pl.ds(c0, _ACC_C), :], max_acc[pl.ds(c0, _ACC_C), :])
                    lo = h0
                s, m = accum(c0, _ACC_C, lo, h0 + n, init)
                sum_acc[pl.ds(c0, _ACC_C), :] = s
                max_acc[pl.ds(c0, _ACC_C), :] = m
                return 0

            lax.fori_loop(0, nc // _ACC_C, cb_body, 0)
            if i == 1:
                w1c.wait()
                w2c.wait()
                row = lax.broadcasted_iota(jnp.int32, (R, 128), 0)
                col = lax.broadcasted_iota(jnp.int32, (R, 128), 1)
                e = jnp.where((col == row) | (col == row + 64), 1.0, 0.0).astype(bf16)
                dn = (((0,), (0,)), ((), ()))
                w1b[...] = lax.dot_general(w1t_v[...], e, dn, preferred_element_type=f32)
                w2b[...] = lax.dot_general(w2_v[...], e, dn, preferred_element_type=f32)

        part = layer1_partial(sum_acc[pl.ds(0, CA), :], max_acc[pl.ds(0, CA), :], 0, CA)
        carry = (sum_acc[pl.ds(CA, _CB), :], max_acc[pl.ds(CA, _CB), :])
        for i in range(n_fa, len(reads)):
            h0, n, _, _ = reads[i]
            in_copy(i).wait()
            carry = accum(CA, _CB, h0, h0 + n, carry)

        part = part + layer1_partial(carry[0], carry[1], CA, _CB)
        hid = jnp.sum(part, axis=0, keepdims=True).astype(bf16).astype(f32)
        hid = jnp.maximum(hid, 0.0)
        z = jnp.sum(w2b[...] * hid, axis=-1, keepdims=True)
        sc = jax.nn.sigmoid(z).astype(bf16).astype(f32)

        o0 = 0
        for n in _FIRST:
            for o in range(o0, o0 + n):
                for (h, c0, nc, r) in segments(0, _PARTS[0] * 8, C):
                    v = xbuf[h + HG * o, pl.ds(c0, nc), :].astype(f32)
                    obuf[o, pl.ds(r, nc), :] = (v * sc[c0:c0 + nc]).astype(obuf.dtype)
            out_copy(0, o0, n).start()
            o0 += n
        scale_v[...] = jnp.broadcast_to(sc, (C, 128))
        k = 1
        while k < len(_PARTS):
            ks = range(k, min(k + (1 if k < 4 else _GROUP), len(_PARTS)))
            scale_rows(p_st[ks[0]] * 8, (p_st[ks[-1]] + _PARTS[ks[-1]]) * 8)
            for kk in ks:
                out_copy(kk, 0, NO).start()
            k = ks[-1] + 1

    pl.run_scoped(main, pltpu.SemaphoreType.DMA((1 + len(reads),)))
    pltpu.make_async_copy(obuf, o_hbm, out_sem.at[0]).wait()


@jax.jit
def pallas_standalone__channel_attn_cbam__vision_kernel(
    x: jax.Array,
    w1: jax.Array,
    w2: jax.Array,
):
    B, H, W, C = x.shape
    r = w1.shape[1]
    NO = H * C // _PER
    assert B == 1 and r <= 64 and 128 < W <= 256
    assert _PER % C == 0 and NO * _PER == H * C and sum(_FIRST) == NO
    assert sum(_F_CHUNKS) + sum(_A_CHUNKS) == H and sum(_A_CHUNKS) == sum(_B_CHUNKS)
    assert C % _ACC_C == 0 and _CB % _ACC_C == 0
    xt = jnp.transpose(x, (0, 1, 3, 2)).reshape(H, C, W)
    out = pl.pallas_call(
        _kernel,
        out_shape=jax.ShapeDtypeStruct((NO, _PER, W), x.dtype),
        in_specs=[pl.BlockSpec(memory_space=pl.ANY)] * 3,
        out_specs=pl.BlockSpec(memory_space=pl.ANY),
        scratch_shapes=[
            pltpu.VMEM((H, C, W), x.dtype),
            pltpu.VMEM((NO, _PER, W), x.dtype),
            pltpu.VMEM((r, C), w1.dtype),
            pltpu.VMEM((r, C), w2.dtype),
            pltpu.VMEM((C, 128), f32),
            pltpu.VMEM((C, 128), f32),
            pltpu.VMEM((C, W), f32),
            pltpu.VMEM((C, W), f32),
            pltpu.VMEM((C, 128), f32),
            pltpu.SemaphoreType.DMA((1,)),
        ],
        compiler_params=pltpu.CompilerParams(vmem_limit_bytes=64 * 1024 * 1024),
    )(xt, w1.T, w2)
    return jnp.transpose(out.reshape(B, H, C, W), (0, 1, 3, 2))
```

```python
import jax
import jax.numpy as jnp
from jax import lax
import jax.experimental.pallas as pl
import jax.experimental.pallas.tpu as pltpu

f32, bf16 = jnp.float32, jnp.bfloat16

_F_CHUNKS = (100, 56, 24, 12)
_A_CHUNKS = (16, 10, 6)
_B_CHUNKS = (20, 8, 3, 1)
_CB = 32
_ACC_C = 32
_UNROLL = 4
_INLINE_MAX = 8
_PARTS = (3, 3, 6) + (7,) * 108
_FIRST = (2, 5)
_GROUP = 3
_PER = sum(_PARTS) * 8


def _starts(chunks, base=0):
    return [base + sum(chunks[:i]) for i in range(len(chunks))]


def _kernel(x_hbm, w1t_hbm, w2_hbm, o_hbm,
            xbuf, obuf, w1t_v, w2_v, w1b, w2b, sum_acc, max_acc, scale_v, out_sem):
    H, C, W = xbuf.shape
    R = w1t_v.shape[0]
    CA = C - _CB
    NO = o_hbm.shape[0]
    HG = _PER // C
    HF = sum(_F_CHUNKS)
    p_st = _starts(_PARTS)
    reads = ([(s, n, 0, C) for s, n in zip(_starts(_F_CHUNKS), _F_CHUNKS)]
             + [(s, n, 0, CA) for s, n in zip(_starts(_A_CHUNKS, HF), _A_CHUNKS)]
             + [(s, n, CA, _CB) for s, n in zip(_starts(_B_CHUNKS, HF), _B_CHUNKS)])
    n_fa = len(_F_CHUNKS) + len(_A_CHUNKS)

    def out_copy(k, o0, n):
        idx = (pl.ds(o0, n), pl.ds(p_st[k] * 8, _PARTS[k] * 8))
        return pltpu.make_async_copy(obuf.at[idx], o_hbm.at[idx], out_sem.at[0])

    def accum(c0, n_c, lo, hi, carry):
        def body(h, carry):
            s, m = carry
            v = xbuf[h, pl.ds(c0, n_c), :].astype(f32)
            return s + v, jnp.maximum(m, v)

        if hi - lo <= _INLINE_MAX:
            for h in range(lo, hi):
                carry = body(h, carry)
            return carry
        return lax.fori_loop(lo, hi, body, carry, unroll=_UNROLL)

    def layer1_partial(s, m, c0, n_c):
        gap = (jnp.sum(s, axis=-1, keepdims=True) * (1.0 / (H * W))).astype(bf16).astype(f32)
        gmp = jnp.max(m, axis=-1, keepdims=True)
        lane = lax.broadcasted_iota(jnp.int32, (n_c, 128), 1)
        prod = jnp.where(lane < 64, gap, gmp) * w1b[pl.ds(c0, n_c), :]
        return jnp.sum(prod.reshape(n_c // 8, 8, 128), axis=0)

    def segments(r, end, max_rows):
        segs = []
        while r < end:
            h, c0 = divmod(r, C)
            n = min(end - r, C - c0, max_rows)
            segs.append((h, c0, n, r))
            r += n
        return segs

    def scale_rows(r0, r1):
        for (h, c0, nc, r) in segments(r0, r1, 88):
            s128 = scale_v[pl.ds(c0, nc), :]
            s = jnp.concatenate([s128, s128[:, :W - 128]], axis=1)
            for o in range(NO):
                v = xbuf[h + HG * o, pl.ds(c0, nc), :].astype(f32)
                obuf[o, pl.ds(r, nc), :] = (v * s).astype(obuf.dtype)

    def main(in_sems):
        def in_copy(i):
            h0, n, c0, nc = reads[i]
            idx = (pl.ds(h0, n),) if nc == C else (pl.ds(h0, n), pl.ds(c0, nc))
            return pltpu.make_async_copy(x_hbm.at[idx], xbuf.at[idx], in_sems.at[1 + i])

        w1c = pltpu.make_async_copy(w1t_hbm, w1t_v, in_sems.at[0])
        w2c = pltpu.make_async_copy(w2_hbm, w2_v, in_sems.at[0])
        in_copy(0).start()
        w1c.start()
        w2c.start()
        in_copy(1).start()

        for i in range(n_fa):
            h0, n, _, nc = reads[i]
            in_copy(i).wait()
            if i == 0:
                for j in range(2, len(reads)):
                    in_copy(j).start()

            def cb_body(j, _, i=i, h0=h0, n=n):
                c0 = pl.multiple_of(j * _ACC_C, _ACC_C)
                if i == 0:
                    v = xbuf[h0, pl.ds(c0, _ACC_C), :].astype(f32)
                    init, lo = (v, v), h0 + 1
                else:
                    init = (sum_acc[pl.ds(c0, _ACC_C), :], max_acc[pl.ds(c0, _ACC_C), :])
                    lo = h0
                s, m = accum(c0, _ACC_C, lo, h0 + n, init)
                sum_acc[pl.ds(c0, _ACC_C), :] = s
                max_acc[pl.ds(c0, _ACC_C), :] = m
                return 0

            lax.fori_loop(0, nc // _ACC_C, cb_body, 0)
            if i == 1:
                w1c.wait()
                w2c.wait()
                row = lax.broadcasted_iota(jnp.int32, (R, 128), 0)
                col = lax.broadcasted_iota(jnp.int32, (R, 128), 1)
                e = jnp.where((col == row) | (col == row + 64), 1.0, 0.0).astype(bf16)
                dn = (((0,), (0,)), ((), ()))
                w1b[...] = lax.dot_general(w1t_v[...], e, dn, preferred_element_type=f32)
                w2b[...] = lax.dot_general(w2_v[...], e, dn, preferred_element_type=f32)

        part = layer1_partial(sum_acc[pl.ds(0, CA), :], max_acc[pl.ds(0, CA), :], 0, CA)
        carry = (sum_acc[pl.ds(CA, _CB), :], max_acc[pl.ds(CA, _CB), :])
        for i in range(n_fa, len(reads)):
            h0, n, _, _ = reads[i]
            in_copy(i).wait()
            carry = accum(CA, _CB, h0, h0 + n, carry)

        part = part + layer1_partial(carry[0], carry[1], CA, _CB)
        hid = jnp.sum(part, axis=0, keepdims=True).astype(bf16).astype(f32)
        hid = jnp.maximum(hid, 0.0)
        z = jnp.sum(w2b[...] * hid, axis=-1, keepdims=True)

        def scale_of(c0, c1):
            return jax.nn.sigmoid(z[c0:c1]).astype(bf16).astype(f32)

        done = _PARTS[0] * 8
        sc = scale_of(0, done)
        o0 = 0
        for n in _FIRST:
            for o in range(o0, o0 + n):
                v = xbuf[HG * o, pl.ds(0, done), :].astype(f32)
                obuf[o, pl.ds(0, done), :] = (v * sc).astype(obuf.dtype)
            out_copy(0, o0, n).start()
            o0 += n
        scale_v[pl.ds(0, done), :] = jnp.broadcast_to(sc, (done, 128))
        k = 1
        while k < len(_PARTS):
            ks = range(k, min(k + (1 if k < 4 else _GROUP), len(_PARTS)))
            r0, r1 = p_st[ks[0]] * 8, (p_st[ks[-1]] + _PARTS[ks[-1]]) * 8
            need = min(C, r1)
            if need > done:
                scale_v[pl.ds(done, need - done), :] = jnp.broadcast_to(
                    scale_of(done, need), (need - done, 128))
                done = need
            scale_rows(r0, r1)
            for kk in ks:
                out_copy(kk, 0, NO).start()
            k = ks[-1] + 1

    pl.run_scoped(main, pltpu.SemaphoreType.DMA((1 + len(reads),)))
    pltpu.make_async_copy(obuf, o_hbm, out_sem.at[0]).wait()


@jax.jit
def pallas_standalone__channel_attn_cbam__vision_kernel(
    x: jax.Array,
    w1: jax.Array,
    w2: jax.Array,
):
    B, H, W, C = x.shape
    r = w1.shape[1]
    NO = H * C // _PER
    assert B == 1 and r <= 64 and 128 < W <= 256
    assert _PER % C == 0 and NO * _PER == H * C and sum(_FIRST) == NO
    assert sum(_F_CHUNKS) + sum(_A_CHUNKS) == H and sum(_A_CHUNKS) == sum(_B_CHUNKS)
    assert C % _ACC_C == 0 and _CB % _ACC_C == 0 and _PARTS[0] * 8 <= C
    xt = jnp.transpose(x, (0, 1, 3, 2)).reshape(H, C, W)
    out = pl.pallas_call(
        _kernel,
        out_shape=jax.ShapeDtypeStruct((NO, _PER, W), x.dtype),
        in_specs=[pl.BlockSpec(memory_space=pl.ANY)] * 3,
        out_specs=pl.BlockSpec(memory_space=pl.ANY),
        scratch_shapes=[
            pltpu.VMEM((H, C, W), x.dtype),
            pltpu.VMEM((NO, _PER, W), x.dtype),
            pltpu.VMEM((r, C), w1.dtype),
            pltpu.VMEM((r, C), w2.dtype),
            pltpu.VMEM((C, 128), f32),
            pltpu.VMEM((C, 128), f32),
            pltpu.VMEM((C, W), f32),
            pltpu.VMEM((C, W), f32),
            pltpu.VMEM((C, 128), f32),
            pltpu.SemaphoreType.DMA((1,)),
        ],
        compiler_params=pltpu.CompilerParams(vmem_limit_bytes=64 * 1024 * 1024),
    )(xt, w1.T, w2)
    return jnp.transpose(out.reshape(B, H, C, W), (0, 1, 3, 2))
```
